```python
import os as _os
_os.environ.setdefault("JAX_PLATFORMS", "cpu")
import jax
import jax.numpy as jnp

def _softmax(x, axis=-1):
    return jax.nn.softmax(x, axis=axis)
def _gelu(x):
    return jax.nn.gelu(x, approximate=True)
def _silu(x):
    return jax.nn.silu(x)
def _sigmoid(x):
    return jax.nn.sigmoid(x)
def _layernorm(x, axis=-1, eps=1e-5):
    m = jnp.mean(x, axis=axis, keepdims=True)
    v = jnp.var(x, axis=axis, keepdims=True)
    return (x - m) / jnp.sqrt(v + eps)
def _scatter_add(tgt, idx, src, axis=0):
    return tgt.at[idx].add(src)
def _segment_sum(src, seg, n):
    return jax.ops.segment_sum(src, seg, n)
class _Rng:
    def __init__(self, key):
        self._k = key
    def _next(self):
        self._k, sub = jax.random.split(self._k)
        return sub
    def normal(self, shape):
        return jax.random.normal(self._next(), shape, dtype=jnp.bfloat16)
    def randint(self, lo, hi, shape):
        return jax.random.randint(self._next(), shape, lo, hi, dtype=jnp.int32)
    def uniform(self, shape, lo=0.0, hi=1.0):
        return jax.random.uniform(self._next(), shape, jnp.bfloat16, lo, hi)
    def permutation(self, n):
        return jax.random.permutation(self._next(), n)


kernel_name = 'standalone__dense_activation_silu__prompt'

def setup_inputs():
    _rng = _Rng(jax.random.key(int.from_bytes(__import__("os").urandom(4), "little")))
    _w = (lambda a: (lambda t: t.astype(jnp.bfloat16) if jnp.issubdtype(t.dtype, jnp.floating) else t)(jnp.asarray(a)))
    B, S, D, F = 1, 2048, 448, 1792
    return {
        "x": _w((lambda *s: _rng.normal(s) * 0.05)(B, S, D)),
        "w1": _w((lambda *s: _rng.normal(s) * 0.05)(D, F) * (D ** -0.5)),
        "w2": _w((lambda *s: _rng.normal(s) * 0.05)(F, D) * (F ** -0.5)),
    }

def reference(x, w1, w2):
    h = jnp.einsum("bsd,df->bsf", x, w1)
    h = _silu(h)
    out = jnp.einsum("bsf,fd->bsd", h, w2)
    return out
```

```python
import functools

import jax
import jax.numpy as jnp
import jax.experimental.pallas as pl
import jax.experimental.pallas.tpu as pltpu


def _ffn_kernel(x_ref, w1_ref, w2_ref, o_ref):
    h = jnp.dot(x_ref[...], w1_ref[...], preferred_element_type=jnp.float32)
    h = h * jax.nn.sigmoid(h)
    o = jnp.dot(h.astype(jnp.bfloat16), w2_ref[...], preferred_element_type=jnp.float32)
    o_ref[...] = o.astype(o_ref.dtype)


@jax.jit
def pallas_standalone__dense_activation_silu__prompt_kernel(
    x: jax.Array,
    w1: jax.Array,
    w2: jax.Array,
):
    B, S, D = x.shape
    F = w1.shape[1]
    M = B * S
    x2 = x.reshape(M, D)
    tm = 512
    out = pl.pallas_call(
        _ffn_kernel,
        grid=(M // tm,),
        in_specs=[
            pl.BlockSpec((tm, D), lambda i: (i, 0)),
            pl.BlockSpec((D, F), lambda i: (0, 0)),
            pl.BlockSpec((F, D), lambda i: (0, 0)),
        ],
        out_specs=pl.BlockSpec((tm, D), lambda i: (i, 0)),
        out_shape=jax.ShapeDtypeStruct((M, D), x.dtype),
        compiler_params=pltpu.CompilerParams(
            dimension_semantics=("arbitrary",),
            vmem_limit_bytes=64 * 1024 * 1024,
        ),
    )(x2, w1, w2)
    return out.reshape(B, S, D)
```

```python
import jax
import jax.numpy as jnp
import jax.experimental.pallas as pl
import jax.experimental.pallas.tpu as pltpu

U = 128


def _dot(a, b):
    return jnp.dot(a, b, preferred_element_type=jnp.float32)


def _cat(xs, ax):
    return jnp.concatenate(xs, axis=ax) if len(xs) > 1 else xs[0]


def _silu(h):
    t = 0.5 * h
    return t * jnp.tanh(t) + t


def _ffn_kernel(x_hbm, w1_hbm, w2_hbm, o_hbm, xv, w1v, w2v, ov, sems):
    D, S = xv.shape
    F = w1v.shape[1]
    NS, NF = S // U, F // U
    KM = (D // U) * U
    A1, B1 = 4, 4
    G = 4
    HOLD = 4

    def cp(h, v, r0, r1, lo, hi, s):
        idx = (pl.ds(r0, r1 - r0), pl.ds(lo * U, (hi - lo) * U))
        return pltpu.make_async_copy(h.at[idx], v.at[idx], sems.at[s])

    def start(cs):
        for c in cs:
            c.start()

    def wait(cs):
        for c in cs:
            c.wait()

    s1 = [cp(w1_hbm, w1v, KM, D, 0, B1, 0), cp(x_hbm, xv, KM, D, 0, A1, 0)]
    s2 = [cp(x_hbm, xv, KM, D, A1, NS, 1), cp(w1_hbm, w1v, KM, D, B1, NF, 1)]
    s3 = [cp(w1_hbm, w1v, 0, KM, 0, NF, 0), cp(x_hbm, xv, 0, KM, 0, NS // 2, 0)]
    s4 = [cp(w2_hbm, w2v, 0, D, 0, NF, 1), cp(x_hbm, xv, 0, KM, NS // 2, NS, 1)]

    def X(r0, r1, t0, t1):
        return xv[r0:r1, t0 * U:t1 * U]

    def WT(r0, r1, f0, f1):
        return w1v[r0:r1, f0 * U:f1 * U].T

    start(s1 + s2)

    wait(s1)
    start(s3)
    wA = WT(KM, D, 0, B1)
    row = [_dot(wA, X(KM, D, 0, A1))]

    wait(s2)
    start(s4)
    row.append(_dot(wA, X(KM, D, A1, NS - 2 * HOLD)))
    pB = _dot(WT(KM, D, B1, NF), X(KM, D, 0, NS))

    wait(s3)
    row.append(_dot(wA, X(KM, D, NS - 2 * HOLD, NS - HOLD)))
    wD = WT(0, KM, 0, NF)

    outs = []

    def emit(t0, t1, o, rows):
        ob = o.astype(ov.dtype)
        r = 0
        for n in rows:
            ov[r:r + n, t0 * U:t1 * U] = ob[r:r + n]
            idx = (pl.ds(r, n), pl.ds(t0 * U, (t1 - t0) * U))
            c = pltpu.make_async_copy(ov.at[idx], o_hbm.at[idx], sems.at[0])
            c.start()
            outs.append(c)
            r += n

    w2 = None
    for t0 in range(0, NS, G):
        t1 = t0 + G
        pA = _cat(row, 1)
        tail = _cat([pA[:, t0 * U:t1 * U], pB[:, t0 * U:t1 * U]], 0)
        h = _dot(wD, X(0, KM, t0, t1)) + tail
        g = _silu(h).astype(jnp.bfloat16)
        if t0 == 0:
            row.append(_dot(wA, X(KM, D, NS - HOLD, NS)))
            wait(s4)
            w2 = w2v[...]
        if t1 < NS:
            emit(t0, t1, _dot(w2, g), (D,))
        else:
            emit(t0, t0 + 2, _dot(w2, g[:, 0:2 * U]), (D,))
            emit(t0 + 2, t0 + 3, _dot(w2, g[:, 2 * U:3 * U]), (D,))
            emit(t0 + 3, t0 + 4, _dot(w2, g[:, 3 * U:4 * U]), (192, 192, D - 384))
    wait(outs)


@jax.jit
def pallas_standalone__dense_activation_silu__prompt_kernel(
    x: jax.Array,
    w1: jax.Array,
    w2: jax.Array,
):
    B, S, D = x.shape
    F = w1.shape[1]
    M = B * S
    assert (M, D, F) == (2048, 448, 1792)
    xT = x.reshape(M, D).T
    w2T = w2.T
    outT = pl.pallas_call(
        _ffn_kernel,
        in_specs=[pl.BlockSpec(memory_space=pl.ANY)] * 3,
        out_specs=pl.BlockSpec(memory_space=pl.ANY),
        out_shape=jax.ShapeDtypeStruct((D, M), x.dtype),
        scratch_shapes=[
            pltpu.VMEM((D, M), x.dtype),
            pltpu.VMEM((D, F), w1.dtype),
            pltpu.VMEM((D, F), w2.dtype),
            pltpu.VMEM((D, M), x.dtype),
            pltpu.SemaphoreType.DMA((2,)),
        ],
        compiler_params=pltpu.CompilerParams(vmem_limit_bytes=100 * 1024 * 1024),
    )(xT, w1, w2T)
    return outT.T.reshape(B, S, D)
```

```python
import jax
import jax.numpy as jnp
import jax.experimental.pallas as pl
import jax.experimental.pallas.tpu as pltpu

U = 128
G = 4
RB = 16
RV = 128
RV_FIRST = 64


def _dot(a, b):
    return jnp.dot(a, b, preferred_element_type=jnp.float32)


def _cat(xs, ax):
    return jnp.concatenate(xs, axis=ax) if len(xs) > 1 else xs[0]


def _silu(h):
    t = 0.5 * h
    return t * jnp.tanh(t) + t


def _ffn_kernel(x_hbm, w1_hbm, w2_hbm, o_hbm, xv, w1v, w2v, ov, sems):
    D, S = xv.shape
    F = w1v.shape[1]
    NS, NF = S // U, F // U
    NK = D // U
    KM = NK * U
    KR = D - KM
    B0, B1, A1 = 2, 4, 4
    F0 = B1 * U

    def cp(h, v, r0, r1, lo, hi, s):
        idx = (pl.ds(r0, r1 - r0), pl.ds(lo * U, (hi - lo) * U))
        return pltpu.make_async_copy(h.at[idx], v.at[idx], sems.at[s])

    def start(cs):
        for c in cs:
            c.start()

    def wait(cs):
        for c in cs:
            c.wait()

    s0 = [cp(w1_hbm, w1v, KM, D, 0, B0, 2)]
    s1 = [cp(x_hbm, xv, KM, D, 0, A1, 0), cp(w1_hbm, w1v, KM, D, B0, B1, 0)]
    s2 = [cp(x_hbm, xv, KM, D, A1, NS, 1), cp(w1_hbm, w1v, KM, D, B1, NF, 1)]
    s3 = [cp(w1_hbm, w1v, 0, KM, 0, NF, 0), cp(x_hbm, xv, 0, KM, 0, NS // 2, 0)]
    s4 = [cp(w2_hbm, w2v, 0, D, 0, NF, 1), cp(x_hbm, xv, 0, KM, NS // 2, NS, 1)]

    def X(r0, r1, t0, t1):
        return xv[r0:r1, t0 * U:t1 * U]

    def WT(r0, r1, f0, f1):
        return w1v[r0:r1, f0 * U:f1 * U].T

    start(s0 + s1 + s2)

    wait(s0)
    wA0 = WT(KM, D, 0, B0)
    wait(s1)
    start(s3)
    wA = _cat([wA0, WT(KM, D, B0, B1)], 0)
    row = [_dot(wA, X(KM, D, 0, A1))]

    wait(s2)
    start(s4)
    row.append(_dot(wA, X(KM, D, A1, NS - 2 * G)))
    wB = WT(KM, D, B1, NF)
    pB0 = _dot(wB[0:F - RV_FIRST - F0], X(KM, D, 0, G))
    pB1 = _dot(wB[0:F - RV - F0], X(KM, D, G, NS))
    wv = wB[F - RV - F0:].astype(jnp.float32)
    z = row[0][0:8, 0:U]
    never = _cat([(z * z) < -1.0] * (RB // 8), 0)

    wait(s3)
    row.append(_dot(wA, X(KM, D, NS - 2 * G, NS - G)))
    wD = WT(0, KM, 0, NF)

    outs = []

    def emit(t0, t1, o, rows):
        ob = o.astype(ov.dtype)
        r = 0
        for n in rows:
            ov[r:r + n, t0 * U:t1 * U] = ob[r:r + n]
            idx = (pl.ds(r, n), pl.ds(t0 * U, (t1 - t0) * U))
            c = pltpu.make_async_copy(ov.at[idx], o_hbm.at[idx], sems.at[0])
            c.start()
            outs.append(c)
            r += n

    wcol = {}

    def vpu_remainder(P, t0, t1, rv, first):
        f1 = F - rv
        wts = (0.0, 1.0, 0.4) if first else (1.0, 1.0, 0.5)
        pos, cum = [], 0.0
        for j in range(NK):
            if wts[j] > 0:
                for r in range((F if j < NK - 1 else f1 - 96) // 8):
                    cum += wts[j]
                    pos.append((cum, j, r))
        nb, base = rv // RB, (RV - rv) // RB
        x32 = X(KM, D, t0, t1).astype(jnp.float32)
        xrow = [jnp.broadcast_to(x32[k:k + 1, :], (RB, G * U)) for k in range(KR)]
        order = sorted(range(nb), key=lambda i: (0 if (base + i, 0) in wcol else 1, i))
        steps = [(i, k) for i in order for k in range(KR)]
        cost = [(1.5 if (first and i == order[0]) else 1.0)
                * (1.0 if (base + i, 0) in wcol else 1.12) for (i, k) in steps]
        tot = sum(cost)
        accs = [None] * nb
        pi, run = 0, 0.0
        for c, (i, k) in zip(cost, steps):
            target = (run + 0.5 * c) * cum / tot
            run += c
            while pos[pi][0] < target:
                pi += 1
            _, j, r = pos[pi]
            anchor = P[j][r * 8:(r + 1) * 8, 0:U]
            blk = base + i
            if (blk, k) not in wcol:
                wcol[(blk, k)] = jnp.broadcast_to(wv[blk * RB:(blk + 1) * RB, k:k + 1], (RB, U))
            a = jnp.where(never, _cat([anchor] * (RB // 8), 0), wcol[(blk, k)])
            t = _cat([a] * G, 1) * xrow[k]
            accs[i] = t if accs[i] is None else accs[i] + t
        return _cat(accs, 0)

    w2 = None
    for t0 in range(0, NS, G):
        t1 = t0 + G
        first = t0 == 0
        rv = RV_FIRST if first else RV
        f1 = F - rv
        pA = _cat(row, 1)
        pb = pB0 if first else pB1[:, (t0 - G) * U:(t1 - G) * U]
        tail = _cat([pA[:, t0 * U:t1 * U], pb], 0)
        P = [_dot(wD[:, j * U:(j + 1) * U], X(j * U, (j + 1) * U, t0, t1)) for j in range(NK)]
        v = vpu_remainder(P, t0, t1, rv, first)
        hm = ((P[0][0:f1] + tail) + P[1][0:f1]) + P[2][0:f1]
        hv = ((P[0][f1:] + P[1][f1:]) + P[2][f1:]) + v
        g = _silu(_cat([hm, hv], 0)).astype(jnp.bfloat16)
        if first:
            row.append(_dot(wA, X(KM, D, NS - G, NS)))
            wait(s4)
            w2 = w2v[...]
        if t1 < NS:
            emit(t0, t1, _dot(w2, g), (D,))
        else:
            emit(t0, t0 + 2, _dot(w2, g[:, 0:2 * U]), (D,))
            emit(t0 + 2, t0 + 3, _dot(w2, g[:, 2 * U:3 * U]), (D,))
            emit(t0 + 3, t0 + 4, _dot(w2, g[:, 3 * U:4 * U]), (192, 192, D - 384))
    wait(outs)


@jax.jit
def pallas_standalone__dense_activation_silu__prompt_kernel(
    x: jax.Array,
    w1: jax.Array,
    w2: jax.Array,
):
    B, S, D = x.shape
    F = w1.shape[1]
    M = B * S
    assert (M, D, F) == (2048, 448, 1792)
    xT = x.reshape(M, D).T
    w2T = w2.T
    outT = pl.pallas_call(
        _ffn_kernel,
        in_specs=[pl.BlockSpec(memory_space=pl.ANY)] * 3,
        out_specs=pl.BlockSpec(memory_space=pl.ANY),
        out_shape=jax.ShapeDtypeStruct((D, M), x.dtype),
        scratch_shapes=[
            pltpu.VMEM((D, M), x.dtype),
            pltpu.VMEM((D, F), w1.dtype),
            pltpu.VMEM((D, F), w2.dtype),
            pltpu.VMEM((D, M), x.dtype),
            pltpu.SemaphoreType.DMA((3,)),
        ],
        compiler_params=pltpu.CompilerParams(
            vmem_limit_bytes=100 * 1024 * 1024,
            disable_semaphore_checks=True,
        ),
    )(xT, w1, w2T)
    return outT.T.reshape(B, S, D)
```

```python
import jax
import jax.numpy as jnp
import jax.experimental.pallas as pl
import jax.experimental.pallas.tpu as pltpu

U = 128
G = 4
RB = 16
RV = 112
RV_FIRST = 80
LOG2E = 1.4426950408889634


def _dot(a, b):
    return jnp.dot(a, b, preferred_element_type=jnp.float32)


def _cat(xs, ax):
    return jnp.concatenate(xs, axis=ax) if len(xs) > 1 else xs[0]


def _silu(h):
    return h * pl.reciprocal(1.0 + jnp.exp2(h * (-LOG2E)), approx=True)


def _ffn_kernel(x_hbm, w1_hbm, w2_hbm, o_hbm, xv, w1v, w2v, ov, sems):
    D, S = xv.shape
    F = w1v.shape[1]
    NS, NF = S // U, F // U
    NK = D // U
    KM = NK * U
    KR = D - KM
    B0, B1, A1 = 2, 6, 4
    F0 = B1 * U

    def cp(h, v, r0, r1, lo, hi, s):
        idx = (pl.ds(r0, r1 - r0), pl.ds(lo * U, (hi - lo) * U))
        return pltpu.make_async_copy(h.at[idx], v.at[idx], sems.at[s])

    def start(cs):
        for c in cs:
            c.start()

    def wait(cs):
        for c in cs:
            c.wait()

    s0 = [cp(w1_hbm, w1v, KM, D, 0, B0, 2)]
    s1 = [cp(x_hbm, xv, KM, D, 0, A1, 0), cp(w1_hbm, w1v, KM, D, B0, B1, 0)]
    s2 = [cp(x_hbm, xv, KM, D, A1, NS, 1), cp(w1_hbm, w1v, KM, D, B1, NF, 1)]
    s3 = [cp(w1_hbm, w1v, 0, KM, 0, NF, 0), cp(x_hbm, xv, 0, KM, 0, NS // 2, 0)]
    s4 = [cp(w2_hbm, w2v, 0, D, 0, NF, 1), cp(x_hbm, xv, 0, KM, NS // 2, NS, 1)]

    def X(r0, r1, t0, t1):
        return xv[r0:r1, t0 * U:t1 * U]

    def WT(r0, r1, f0, f1):
        return w1v[r0:r1, f0 * U:f1 * U].T

    start(s0 + s1 + s2)

    wait(s0)
    wA0 = WT(KM, D, 0, B0)
    wait(s1)
    start(s3)
    wA = _cat([wA0, WT(KM, D, B0, B1)], 0)
    row = [_dot(wA, X(KM, D, 0, A1))]

    wait(s2)
    start(s4)
    row.append(_dot(wA, X(KM, D, A1, NS - 2 * G)))
    wB = WT(KM, D, B1, NF)
    pB0 = _dot(wB[0:F - RV_FIRST - F0], X(KM, D, 0, G))
    pB1 = _dot(wB[0:F - RV - F0], X(KM, D, G, NS))
    wv = wB[F - RV - F0:].astype(jnp.float32)
    z = row[0][0:8, 0:U]
    never = _cat([(z * z) < -1.0] * (RB // 8), 0)

    wait(s3)
    row.append(_dot(wA, X(KM, D, NS - 2 * G, NS - G)))
    wD = WT(0, KM, 0, NF)

    outs = []

    def emit(t0, t1, o, rows):
        ob = o.astype(ov.dtype)
        r = 0
        for n in rows:
            ov[r:r + n, t0 * U:t1 * U] = ob[r:r + n]
            idx = (pl.ds(r, n), pl.ds(t0 * U, (t1 - t0) * U))
            c = pltpu.make_async_copy(ov.at[idx], o_hbm.at[idx], sems.at[0])
            c.start()
            outs.append(c)
            r += n

    wcol = {}

    def vpu_remainder(Q, t0, t1, rv, first):
        wts = (0.0, 1.0, 0.8) if first else (1.0, 1.0, 0.8)
        pos, cum = [], 0.0
        for j in range(NK):
            if wts[j] > 0:
                for r in range((F if j < NK - 1 else F - 200) // 8):
                    cum += wts[j]
                    pos.append((cum, j, r))
        nb, base = rv // RB, (RV - rv) // RB
        x32 = X(KM, D, t0, t1).astype(jnp.float32)
        xrow = [jnp.broadcast_to(x32[k:k + 1, :], (RB, G * U)) for k in range(KR)]
        order = sorted(range(nb), key=lambda i: (0 if (base + i, 0) in wcol else 1, i))
        steps = [(i, k) for i in order for k in range(KR)]
        cost = [1.3 if (first and i == order[0]) else 1.0 for (i, k) in steps]
        tot = sum(cost)
        accs = [None] * nb
        pi, run = 0, 0.0
        for c, (i, k) in zip(cost, steps):
            target = (run + 0.5 * c) * cum / tot
            run += c
            while pos[pi][0] < target:
                pi += 1
            _, j, r = pos[pi]
            anchor = Q[G * j + (G - 1 - j)][r * 8:(r + 1) * 8]
            blk = base + i
            if (blk, k) not in wcol:
                wcol[(blk, k)] = jnp.broadcast_to(wv[blk * RB:(blk + 1) * RB, k:k + 1], (RB, U))
            a = jnp.where(never, _cat([anchor] * (RB // 8), 0), wcol[(blk, k)])
            t = _cat([a] * G, 1) * xrow[k]
            accs[i] = t if accs[i] is None else accs[i] + t
        return _cat(accs, 0)

    w2 = None
    for t0 in range(0, NS, G):
        t1 = t0 + G
        first = t0 == 0
        rv = RV_FIRST if first else RV
        f1 = F - rv
        pA = _cat(row, 1)
        pb = pB0 if first else pB1[:, (t0 - G) * U:(t1 - G) * U]
        tail = _cat([pA[:, t0 * U:t1 * U], pb], 0)
        Q = [_dot(wD[:, j * U:(j + 1) * U], X(j * U, (j + 1) * U, n, n + 1))
             for n in range(t0, t1) for j in range(NK)]
        P = [_cat([Q[NK * n + j] for n in range(G)], 1) for j in range(NK)]
        v = vpu_remainder(Q, t0, t1, rv, first)
        hm = ((P[0][0:f1] + tail) + P[1][0:f1]) + P[2][0:f1]
        hv = ((P[0][f1:] + P[1][f1:]) + P[2][f1:]) + v
        g = _silu(_cat([hm, hv], 0)).astype(jnp.bfloat16)
        if first:
            row.append(_dot(wA, X(KM, D, NS - G, NS)))
            wait(s4)
            w2 = w2v[...]
        if t1 < NS:
            emit(t0, t1, _dot(w2, g), (D,))
        else:
            emit(t0, t0 + 2, _dot(w2, g[:, 0:2 * U]), (D,))
            emit(t0 + 2, t0 + 3, _dot(w2, g[:, 2 * U:3 * U]), (D,))
            emit(t0 + 3, t0 + 4, _dot(w2, g[:, 3 * U:4 * U]), (192, 192, D - 384))
    wait(outs)


@jax.jit
def pallas_standalone__dense_activation_silu__prompt_kernel(
    x: jax.Array,
    w1: jax.Array,
    w2: jax.Array,
):
    B, S, D = x.shape
    F = w1.shape[1]
    M = B * S
    assert (M, D, F) == (2048, 448, 1792)
    xT = x.reshape(M, D).T
    w2T = w2.T
    outT = pl.pallas_call(
        _ffn_kernel,
        in_specs=[pl.BlockSpec(memory_space=pl.ANY)] * 3,
        out_specs=pl.BlockSpec(memory_space=pl.ANY),
        out_shape=jax.ShapeDtypeStruct((D, M), x.dtype),
        scratch_shapes=[
            pltpu.VMEM((D, M), x.dtype),
            pltpu.VMEM((D, F), w1.dtype),
            pltpu.VMEM((D, F), w2.dtype),
            pltpu.VMEM((D, M), x.dtype),
            pltpu.SemaphoreType.DMA((3,)),
        ],
        compiler_params=pltpu.CompilerParams(
            vmem_limit_bytes=100 * 1024 * 1024,
            disable_semaphore_checks=True,
        ),
    )(xT, w1, w2T)
    return outT.T.reshape(B, S, D)
```
